```python
import jax
import jax.numpy as jnp

def _softmax(x, axis=-1):
    return jax.nn.softmax(x, axis=axis)

def _gelu(x):
    return jax.nn.gelu(x, approximate=True)

def _silu(x):
    return jax.nn.silu(x)

def _sigmoid(x):
    return jax.nn.sigmoid(x)

def _layernorm(x, axis=-1, eps=1e-05):
    m = jnp.mean(x, axis=axis, keepdims=True)
    v = jnp.var(x, axis=axis, keepdims=True)
    return (x - m) / jnp.sqrt(v + eps)

def _scatter_add(tgt, idx, src, axis=0):
    return tgt.at[idx].add(src)

def _segment_sum(src, seg, n):
    return jax.ops.segment_sum(src, seg, n)

class _Rng:

    def __init__(self, key):
        self._k = key

    def _next(self):
        self._k, sub = jax.random.split(self._k)
        return sub

    def normal(self, shape):
        return jax.random.normal(self._next(), shape, dtype=jnp.bfloat16)

    def randint(self, lo, hi, shape):
        return jax.random.randint(self._next(), shape, lo, hi, dtype=jnp.int32)

    def uniform(self, shape, lo=0.0, hi=1.0):
        return jax.random.uniform(self._next(), shape, jnp.bfloat16, lo, hi)

    def permutation(self, n):
        return jax.random.permutation(self._next(), n)
kernel_name = 'gated_mix__memory_aug_recurrent_mem_tr__moe_arch_mod__prompt'

def setup_inputs():
    _rng = _Rng(jax.random.key(int.from_bytes(__import__("os").urandom(4), "little")))
    _w = lambda a: (lambda t: t.astype(jnp.bfloat16) if jnp.issubdtype(t.dtype, jnp.floating) else t)(jnp.asarray(a))

    def _A_setup():
        B, S, Dm = (1, 2048, 1024)
        H, Dh = (32, 128)
        M, seg = (8, 32)
        seg = min(seg, S)
        S = S // seg * seg
        return {'x': _w((lambda *s: _rng.normal(s) * 0.05)(B, S, Dm)), 'mem0': _w((lambda *s: _rng.normal(s) * 0.05)(B, M, Dm)), 'Wq': _w((lambda *s: _rng.normal(s) * 0.05)(Dm, H, Dh) * Dm ** (-0.5)), 'Wk': _w((lambda *s: _rng.normal(s) * 0.05)(Dm, H, Dh) * Dm ** (-0.5)), 'Wv': _w((lambda *s: _rng.normal(s) * 0.05)(Dm, H, Dh) * Dm ** (-0.5)), 'Wo': _w((lambda *s: _rng.normal(s) * 0.05)(H, Dh, Dm) * (H * Dh) ** (-0.5)), 'seg_len': seg}
    _A_in = _A_setup()

    def _B_setup():
        B, S, D, F, C = (1, 2048, 1024, 3584, 8)
        return {'x': _w((lambda *s: _rng.normal(s) * 0.05)(B, S, D)), 'w_r': _w((lambda *s: _rng.normal(s) * 0.05)(D)), 'w_gate': _w((lambda *s: _rng.normal(s) * 0.05)(D, F)), 'w_up': _w((lambda *s: _rng.normal(s) * 0.05)(D, F)), 'w_down': _w((lambda *s: _rng.normal(s) * 0.05)(F, D))}
    _B_in = _B_setup()
    return {'A_x': _A_in['x'], 'A_mem0': _A_in['mem0'], 'A_Wq': _A_in['Wq'], 'A_Wk': _A_in['Wk'], 'A_Wv': _A_in['Wv'], 'A_Wo': _A_in['Wo'], 'A_seg_len': _A_in['seg_len'], 'B_x': _B_in['x'], 'B_w_r': _B_in['w_r'], 'B_w_gate': _B_in['w_gate'], 'B_w_up': _B_in['w_up'], 'B_w_down': _B_in['w_down'], 'gate_w': _w((lambda *s: _rng.normal(s) * 0.05)(1024))}

def reference(A_x, A_mem0, A_Wq, A_Wk, A_Wv, A_Wo, A_seg_len, B_x, B_w_r, B_w_gate, B_w_up, B_w_down, gate_w):

    def _A_ref(x, mem0, Wq, Wk, Wv, Wo, seg_len):
        B, S, Dm = x.shape
        H, Dh = (Wq.shape[1], Wq.shape[2])
        M = mem0.shape[1]
        scale = Dh ** (-0.5)
        n_seg = S // seg_len
        L = M + seg_len
        idx = jnp.arange(L)
        mask = (idx[:, None] < M) | (idx[:, None] >= idx[None, :])
        mem = mem0
        outs = []
        for s in range(n_seg):
            xs = x[:, s * seg_len:(s + 1) * seg_len, :].copy()
            h = jnp.concatenate([mem, xs], axis=1)
            q = jnp.einsum('btd,dhe->bhte', h, Wq)
            k = jnp.einsum('btd,dhe->bhte', h, Wk)
            v = jnp.einsum('btd,dhe->bhte', h, Wv)
            scores = jnp.einsum('bhqe,bhke->bhqk', q, k) * scale
            scores = jnp.where(mask[None, None], scores, -1000000000.0)
            p = _softmax(scores, axis=-1)
            o = jnp.einsum('bhqk,bhke->bhqe', p, v)
            o = jnp.einsum('bhte,hed->btd', o, Wo)
            mem = o[:, :M, :].copy()
            outs.append(o[:, M:, :])
        return jnp.concatenate(outs, axis=1)

    def _B_ref(x, w_r, w_gate, w_up, w_down):
        B, S, D = x.shape
        C = 8
        r = x @ w_r
        idx = jnp.argsort(-r, axis=-1)[:, :C]
        idx_e = jnp.repeat(idx.reshape(B, C, 1), D, axis=2)
        x_sel = jnp.take_along_axis(x, idx_e, axis=1)
        g = _silu(x_sel @ w_gate)
        u = x_sel @ w_up
        y = g * u @ w_down
        r_sel = _sigmoid(jnp.take_along_axis(r, idx, axis=1))
        y = y * r_sel.reshape(B, C, 1)
        b_off = (jnp.arange(B) * S).reshape(B, 1)
        flat_idx = (idx + b_off).reshape(B * C)
        zero = (x * 0.0).reshape(B * S, D)
        upd = _scatter_add(zero, flat_idx, y.reshape(B * C, D), axis=0)
        return x + upd.reshape(B, S, D)
    x = A_x
    g = _sigmoid((x * gate_w).sum(-1, keepdims=True))
    a = _A_ref(x, A_mem0, A_Wq, A_Wk, A_Wv, A_Wo, A_seg_len)
    b = _B_ref(x, B_w_r, B_w_gate, B_w_up, B_w_down)
    return g * a + (1 - g) * b
```

```python
import jax
import jax.numpy as jnp
from jax import lax
from jax.experimental import pallas as pl
from jax.experimental.pallas import tpu as pltpu

F32, BF16, I32 = jnp.float32, jnp.bfloat16, jnp.int32

LANES = 128
TOPK = 8
KCHUNK = 256
NSLOT = 4
HGROUP = 4
LAG = 8


def _dot(a, b):
    return lax.dot_general(a, b, (((1,), (0,)), ((), ())), preferred_element_type=F32)


def _dot_nt(a, b):
    return lax.dot_general(a, b, (((1,), (1,)), ((), ())), preferred_element_type=F32)


def _bf16(words):
    return pltpu.bitcast(words, BF16)


def _sigmoid(z):
    return 1.0 / (1.0 + jnp.exp(-z))


def _kernel(
    x_hbm, mem0_ref, wq_hbm, wk_hbm, wv_hbm, wo_hbm, wr_ref, wg_hbm, wu_hbm, wd_hbm, gw_ref,
    out_hbm,
    w_s, wo_s, stage_s, xh_s, xb_s, bulk_s, x_s, lhs_s, qkv_s, o_s, acc_s, a_s, out_s,
    wg_s, wu_s, wd_s, h_s, idx_s,
    stage_sem, x_sem, wo_sem, ffn_sem, out_sem,
):
    n_seg, seg, d_model = x_hbm.shape
    n_heads = w_s.shape[1]
    n_mem = mem0_ref.shape[0]
    rows = n_mem + seg
    n_ffn = wg_s.shape[0]
    n_dt = d_model // LANES
    chunks_per_w = d_model // KCHUNK
    n_chunks = 3 * chunks_per_w
    chunk_rows = KCHUNK * n_heads
    scale = LANES ** -0.5

    def stage_copy(w_hbm, c):
        src = w_hbm.at[pl.ds((c % chunks_per_w) * chunk_rows, chunk_rows)]
        return pltpu.make_async_copy(src, stage_s.at[c % NSLOT], stage_sem.at[c % NSLOT])

    def start_stage(c):
        for m, w_hbm in enumerate((wq_hbm, wk_hbm, wv_hbm)):
            @pl.when(c // chunks_per_w == m)
            def _(w_hbm=w_hbm):
                stage_copy(w_hbm, c).start()

    def column_copy(src_hbm, dst, sem, j):
        return pltpu.make_async_copy(
            src_hbm.at[:, pl.ds(pl.multiple_of(j * LANES, LANES), LANES)], dst.at[j], sem)

    head_copy = pltpu.make_async_copy(x_hbm.at[:, pl.ds(0, n_mem)], xh_s, x_sem.at[0])
    x_copy = pltpu.make_async_copy(x_hbm, x_s, x_sem.at[1])
    b_copy = pltpu.make_async_copy(x_hbm, out_s.at[pl.ds(0, n_seg)], x_sem.at[2])

    def out_copy(e):
        return pltpu.make_async_copy(out_s.at[e], out_hbm.at[e], out_sem.at[0])

    head_copy.start()
    for c in range(NSLOT - 1):
        stage_copy(wq_hbm, c).start()
    a_s[...] = jnp.zeros(a_s.shape, F32)
    out_s[n_seg] = jnp.zeros((seg, d_model), BF16)
    head_copy.wait()
    for kc in range(chunks_per_w):
        xh = xh_s[:, :, kc * KCHUNK:(kc + 1) * KCHUNK].astype(F32)
        xb_s[kc] = xh.reshape(n_seg * n_mem, KCHUNK)

    stage_words = stage_s.bitcast(I32)

    def bulk_body(c, carry):
        m, kc, slot = c // chunks_per_w, c % chunks_per_w, c % NSLOT

        @pl.when(c + NSLOT - 1 < n_chunks)
        def _():
            start_stage(c + NSLOT - 1)

        @pl.when(jnp.logical_and(c >= 2, c < 2 + n_dt))
        def _():
            column_copy(wo_hbm, wo_s, wo_sem.at[0], c - 2).start()

        @pl.when(c == 2 + n_dt)
        def _():
            x_copy.start()

        stage_copy(wq_hbm, c).wait()
        krows = pl.ds(pl.multiple_of(kc * (KCHUNK // 2), KCHUNK // 2), KCHUNK // 2)
        for p in range(n_heads // 2):
            words = stage_words[slot, pl.ds(p, KCHUNK, stride=n_heads // 2), :]
            even = pltpu.bitcast(words << 16, F32).astype(BF16)
            odd = pltpu.bitcast(words & -65536, F32).astype(BF16)
            w_s[m, 2 * p, krows, :] = pltpu.bitcast(even, I32)
            w_s[m, 2 * p + 1, krows, :] = pltpu.bitcast(odd, I32)
            part = _dot(xb_s[kc], jnp.concatenate([even, odd], axis=1))
            for t in range(2):
                prev = jnp.where(kc > 0, bulk_s[m, 2 * p + t], 0.0)
                bulk_s[m, 2 * p + t] = prev + part[:, t * LANES:(t + 1) * LANES]
        return carry

    lax.fori_loop(0, n_chunks, bulk_body, 0)

    b_copy.start()

    def start_ffn(j, carry):
        column_copy(wg_hbm, wg_s, ffn_sem.at[0], j).start()
        column_copy(wu_hbm, wu_s, ffn_sem.at[1], j).start()
        return carry

    lax.fori_loop(0, n_ffn, start_ffn, 0)
    for j in range(n_dt):
        column_copy(wd_hbm, wd_s, ffn_sem.at[2], j).start()

    x_copy.wait()
    pltpu.make_async_copy(wo_s, wo_s, wo_sem.at[0]).wait()
    wo_words = wo_s.bitcast(I32)
    lhs_s[0:n_mem] = mem0_ref[...].astype(F32)

    def routed_ffn():
        w_r = jnp.broadcast_to(wr_ref[...].astype(F32), (8, d_model)).astype(BF16)
        n_tok = n_seg * seg
        r_row = _dot_nt(w_r, x_s[...].reshape(n_tok, d_model))
        width = n_tok // 8
        sub = lax.broadcasted_iota(I32, (8, width), 0)
        r = r_row[:, :width]
        for i in range(1, 8):
            r = jnp.where(sub == i, r_row[:, i * width:(i + 1) * width], r)
        r = r.astype(BF16).astype(F32)
        key = jnp.where(r == r, r, -jnp.inf)
        tok = (sub * width + lax.broadcasted_iota(I32, (8, width), 1)).astype(F32)
        free = tok
        slot_id = lax.broadcasted_iota(I32, (TOPK, LANES), 0)
        r_sel = jnp.zeros((TOPK, LANES), F32)
        for i in range(TOPK):
            best = jnp.max(jnp.where(free < n_tok, key, -jnp.inf), keepdims=True)
            pick = jnp.min(jnp.where(key == best, free, float(n_tok)), keepdims=True)
            r_pick = jnp.sum(jnp.where(tok == pick, r, 0.0), keepdims=True)
            r_sel = jnp.where(slot_id == i, r_pick, r_sel)
            free = jnp.where(tok == pick, float(n_tok), free)
            idx_s[i] = jnp.clip(pick.astype(I32)[0, 0], 0, n_tok - 1)

        row_id = lax.broadcasted_iota(I32, (seg, d_model), 0)
        slot_wide = lax.broadcasted_iota(I32, (TOPK, d_model), 0)
        x_sel = jnp.zeros((TOPK, d_model), F32)
        for i in range(TOPK):
            t = idx_s[i]
            blk = jnp.where(row_id == t % seg, x_s[t // seg].astype(F32), 0.0)
            x_sel = jnp.where(slot_wide == i, jnp.sum(blk, axis=0, keepdims=True), x_sel)

        pltpu.make_async_copy(wg_s, wg_s, ffn_sem.at[0]).wait()
        pltpu.make_async_copy(wu_s, wu_s, ffn_sem.at[1]).wait()
        pltpu.make_async_copy(wd_s, wd_s, ffn_sem.at[2]).wait()
        b_copy.wait()
        wg_words, wu_words, wd_words = wg_s.bitcast(I32), wu_s.bitcast(I32), wd_s.bitcast(I32)
        for j in range(n_ffn):
            gate = _dot(x_sel, _bf16(wg_words[j]))
            up = _dot(x_sel, _bf16(wu_words[j]))
            h_s[:, j * LANES:(j + 1) * LANES] = gate * _sigmoid(gate) * up
        y = jnp.concatenate([_dot(h_s[...], _bf16(wd_words[j])) for j in range(n_dt)], axis=1)
        y = y * _sigmoid(r_sel[:, 0:1])
        for i in range(TOPK):
            t = idx_s[i]
            blk = out_s[t // seg].astype(F32)
            out_s[t // seg] = jnp.where(row_id == t % seg, blk + y[i:i + 1], blk).astype(BF16)

    def finish(a, x_idx, out_idx):
        x = x_s[x_idx].astype(F32)
        g = _sigmoid(jnp.sum(x * gw_ref[...].astype(F32), axis=-1, keepdims=True))
        b = out_s[out_idx].astype(F32)
        out_s[out_idx] = (g * a + (1.0 - g) * b).astype(BF16)

    def step(s, carry):
        @pl.when(s == LAG)
        def _():
            routed_ffn()

        lhs_s[n_mem:] = x_s[s].astype(F32)[n_mem:]
        bulk_rows = pl.ds(pl.multiple_of(s * n_mem, n_mem), n_mem)
        qi = lax.broadcasted_iota(I32, (rows, rows), 0)
        ki = lax.broadcasted_iota(I32, (rows, rows), 1)
        mask = jnp.logical_or(qi < n_mem, qi >= ki)

        def project(m, g):
            for h in range(g * HGROUP, (g + 1) * HGROUP):
                qkv_s[m, h] = _dot(lhs_s[...], _bf16(w_s[m, h]))

        def load(m, h):
            return jnp.concatenate(
                [qkv_s[m, h, 0:n_mem], bulk_s[m, h, bulk_rows], qkv_s[m, h, n_mem:]], axis=0)

        def scores(g):
            res = []
            for h in range(g * HGROUP, (g + 1) * HGROUP):
                t = jnp.where(mask, _dot_nt(load(0, h), load(1, h)) * scale, -1e9)
                e = jnp.exp(t - jnp.max(t, axis=-1, keepdims=True))
                res.append((e, 1.0 / jnp.sum(e, axis=-1, keepdims=True)))
            return res

        def attend(g, probs):
            for h, (e, inv) in zip(range(g * HGROUP, (g + 1) * HGROUP), probs):
                o_s[:, h * LANES:(h + 1) * LANES] = _dot(e, load(2, h)) * inv

        def out_proj(h0, h1, j):
            w = _bf16(wo_words[j, h0 * LANES // 2:h1 * LANES // 2])
            return _dot(o_s[:, h0 * LANES:h1 * LANES], w)

        e_idx = jnp.maximum(s - LAG, 0)
        finish(a_s[s % LAG], e_idx, jnp.where(s >= LAG, e_idx, n_seg))

        n_groups = n_heads // HGROUP
        probs = None
        for g in range(n_groups):
            project(0, g)
            project(1, g)
            if g > 0:
                attend(g - 1, probs)
            project(2, g)
            probs = scores(g)
        half = n_heads // 2
        for j in range(n_dt):
            acc_s[:, j * LANES:(j + 1) * LANES] = out_proj(0, half, j)
            if j == n_dt // 2 - 1:
                attend(n_groups - 1, probs)
        for j in range(n_dt):
            cols = slice(j * LANES, (j + 1) * LANES)
            res = acc_s[:, cols] + out_proj(half, n_heads, j)
            lhs_s[0:n_mem, cols] = res[0:n_mem]
            a_s[s % LAG, :, cols] = res[n_mem:]

        @pl.when(s >= LAG)
        def _():
            out_copy(s - LAG).start()

        return carry

    lax.fori_loop(0, n_seg, step, 0)

    for e in range(n_seg - LAG, n_seg):
        finish(a_s[e % LAG], e, e)
        out_copy(e).start()
    done = out_s.at[pl.ds(0, n_seg)]
    pltpu.make_async_copy(done, done, out_sem.at[0]).wait()


def pallas_gated_mix__memory_aug_recurrent_mem_tr__moe_arch_mod__prompt_kernel(
    A_x, A_mem0, A_Wq, A_Wk, A_Wv, A_Wo, A_seg_len,
    B_x, B_w_r, B_w_gate, B_w_up, B_w_down, gate_w,
):
    del B_x
    seg = int(A_seg_len)
    batch, n_tok, d_model = A_x.shape
    _, n_heads, d_head = A_Wq.shape
    n_mem = A_mem0.shape[1]
    d_ffn = B_w_gate.shape[1]
    n_seg = n_tok // seg
    assert batch == 1 and d_head == LANES and n_mem == 8 and seg == 32
    n_dt, n_ffn = d_model // LANES, d_ffn // LANES

    hbm = pl.BlockSpec(memory_space=pl.ANY)
    vmem = pl.BlockSpec(memory_space=pltpu.VMEM)
    out = pl.pallas_call(
        _kernel,
        out_shape=jax.ShapeDtypeStruct((n_seg, seg, d_model), BF16),
        in_specs=[hbm, vmem, hbm, hbm, hbm, hbm, vmem, hbm, hbm, hbm, vmem],
        out_specs=hbm,
        scratch_shapes=[
            pltpu.VMEM((3, n_heads, d_model // 2, LANES), I32),
            pltpu.VMEM((n_dt, n_heads * LANES, LANES), BF16),
            pltpu.VMEM((NSLOT, KCHUNK * n_heads, LANES), BF16),
            pltpu.VMEM((n_seg, n_mem, d_model), BF16),
            pltpu.VMEM((d_model // KCHUNK, n_seg * n_mem, KCHUNK), F32),
            pltpu.VMEM((3, n_heads, n_seg * n_mem, LANES), F32),
            pltpu.VMEM((n_seg, seg, d_model), BF16),
            pltpu.VMEM((seg, d_model), F32),
            pltpu.VMEM((3, n_heads, seg, LANES), F32),
            pltpu.VMEM((n_mem + seg, n_heads * LANES), F32),
            pltpu.VMEM((n_mem + seg, d_model), F32),
            pltpu.VMEM((LAG, seg, d_model), F32),
            pltpu.VMEM((n_seg + 1, seg, d_model), BF16),
            pltpu.VMEM((n_ffn, d_model, LANES), BF16),
            pltpu.VMEM((n_ffn, d_model, LANES), BF16),
            pltpu.VMEM((n_dt, d_ffn, LANES), BF16),
            pltpu.VMEM((TOPK, d_ffn), F32),
            pltpu.SMEM((TOPK,), I32),
            pltpu.SemaphoreType.DMA((NSLOT,)),
            pltpu.SemaphoreType.DMA((3,)),
            pltpu.SemaphoreType.DMA((1,)),
            pltpu.SemaphoreType.DMA((3,)),
            pltpu.SemaphoreType.DMA((1,)),
        ],
        compiler_params=pltpu.CompilerParams(vmem_limit_bytes=120 * 1024 * 1024),
    )(
        A_x.reshape(n_seg, seg, d_model),
        A_mem0.reshape(n_mem, d_model),
        A_Wq.reshape(d_model * n_heads, d_head),
        A_Wk.reshape(d_model * n_heads, d_head),
        A_Wv.reshape(d_model * n_heads, d_head),
        A_Wo.reshape(n_heads * d_head, d_model),
        B_w_r.reshape(1, d_model),
        B_w_gate,
        B_w_up,
        B_w_down,
        gate_w.reshape(1, d_model),
    )
    return out.reshape(batch, n_tok, d_model)
```

```python
import functools

import jax
import jax.numpy as jnp
from jax import lax
from jax.experimental import pallas as pl
from jax.experimental.pallas import tpu as pltpu

F32, BF16, I32 = jnp.float32, jnp.bfloat16, jnp.int32

LANES = 128
N_MXU = 4
TOPK = 8
HEAD = 0
UNROLL = 4
TAIL = 12


def _dot(a, b):
    return lax.dot_general(a, b, (((1,), (0,)), ((), ())), preferred_element_type=F32)


def _dot_nt(a, b):
    return lax.dot_general(a, b, (((1,), (1,)), ((), ())), preferred_element_type=F32)


def _bf16(words):
    return pltpu.bitcast(words, BF16)


def _aligned(start, size):
    return pl.ds(start if isinstance(start, int) else pl.multiple_of(start, size), size)


def _tile(j):
    return slice(j * LANES, (j + 1) * LANES)


def _sigmoid(z):
    return 1.0 / (1.0 + jnp.exp(-z))


def _kernel(
    x_hbm, mem0_hbm, wq_hbm, wk_hbm, wv_hbm, wo_hbm, wr_hbm, wg_hbm, wu_hbm, wd_hbm, gw_hbm,
    out_hbm,
    w_s, wo_s, stage_s, xh_s, bulk_s, x_s, lhs_s, a_s, gate_s, out_s,
    mem0_s, wr_s, gw_s, vec_s, r_s, sel_s, h_s, idx_s, sem, order_sem,
):
    n_seg, seg, d_model = x_hbm.shape
    n_tok = n_seg * seg
    n_heads = w_s.shape[1]
    n_mem = mem0_hbm.shape[0]
    d_ffn = wd_hbm.shape[0]
    n_dt, n_ft = d_model // LANES, d_ffn // LANES
    rows = n_mem + seg
    pairs = n_heads // 2
    scale = LANES ** -0.5

    def weight_copy(m, lo, hi):
        return (wq_hbm, wk_hbm, wv_hbm)[m].at[lo:hi], stage_s.at[m * n_dt + lo:m * n_dt + hi]

    def half_copy(j, i):
        half = pl.ds(i * LANES * pairs, LANES * pairs)
        return wq_hbm.at[j, half], stage_s.at[j, half]

    def head_copies(lo, hi):
        return [(x_hbm.at[:, :n_mem, _tile(j)], xh_s.at[j]) for j in range(lo, hi)]

    def x_copy(i):
        segs = pl.ds(i * n_seg // 4, n_seg // 4)
        return x_hbm.at[segs], x_s.at[segs]

    def wo_copies(lo, hi):
        return [(wo_hbm.at[:, _tile(j)], wo_s.at[j]) for j in range(lo, hi)]

    def ffn_slot(i, j):
        if i == 2:
            return 2 * n_dt + j, 0
        slab, k = divmod(i * n_ft + j, LANES * n_heads // d_model)
        return slab, k * d_model

    def ffn_copies(i, w_hbm):
        depth, width = w_hbm.shape
        slots = [ffn_slot(i, j) for j in range(width // LANES)]
        return [(w_hbm.at[:, _tile(j)], stage_s.at[slab, pl.ds(row, depth)])
                for j, (slab, row) in enumerate(slots)]

    batches = [
        [weight_copy(0, 0, 1)] + head_copies(0, 1),
        [weight_copy(0, 1, 2), half_copy(2, 0)] + head_copies(1, 2),
        [half_copy(2, 1), weight_copy(0, 3, 4)] + head_copies(2, 4),
        [weight_copy(0, 4, 7)] + head_copies(4, 6),
        [weight_copy(0, 7, 8), weight_copy(1, 0, 2)] + head_copies(6, 8)
        + [(mem0_hbm, mem0_s), (wr_hbm, wr_s), (gw_hbm, gw_s)],
        [weight_copy(1, 2, 4), x_copy(0)],
        [weight_copy(1, 4, 8), x_copy(1)],
        [weight_copy(2, 0, 4), x_copy(2)] + wo_copies(0, 2),
        [weight_copy(2, 4, 8), x_copy(3)] + wo_copies(2, 3),
        wo_copies(3, n_dt),
        ffn_copies(0, wg_hbm) + ffn_copies(1, wu_hbm) + ffn_copies(2, wd_hbm),
    ]

    def copies(i):
        return [pltpu.make_async_copy(src, dst, sem.at[i]) for src, dst in batches[i]]

    def advance(i, lo, hi):
        for c in range(lo, hi):
            @pl.when(i == c)
            def _(c=c):
                *most, rest = copies(c)
                for copy in most:
                    copy.wait()
                for copy in copies(c + 1) if c + 2 < len(batches) else ():
                    copy.start()
                rest.wait()

    def out_copy(lo, hi):
        return pltpu.make_async_copy(out_s.at[lo:hi], out_hbm.at[lo:hi], sem.at[len(batches)])

    stage_words = stage_s.bitcast(I32)
    wo_words = wo_s.bitcast(I32)

    def bulk(k0, depth, side=()):
        m, lo = k0 // d_model, k0 % d_model
        side = iter(side)

        def xh(a, b):
            return jnp.concatenate(
                [xh_s[lo // LANES + j].reshape(n_seg * n_mem, LANES)
                 for j in range(a // LANES, b // LANES)], axis=1)

        for p in range(pairs):
            words = jnp.concatenate(
                [stage_words[k0 // LANES + j, pl.ds(p, LANES, stride=pairs), :]
                 for j in range(depth // LANES)], axis=0)
            w = [pltpu.bitcast(half, F32).astype(BF16) for half in (words << 16, words & -65536)]
            if p == 0 or depth < N_MXU * LANES:
                both = None
                for a in range(0, depth, 2 * LANES):
                    b = min(a + 2 * LANES, depth)
                    part = _dot(xh(a, b), jnp.concatenate(w, axis=1)[a:b])
                    both = part if both is None else part + both
                new = [both[:, _tile(t)] for t in range(2)]
            else:
                new = [_dot(xh(0, depth), w[0])]
                next(side, None)
                new.append(_dot(xh(0, depth), w[1]))
            for t in range(2):
                h = 2 * p + t
                w_s[m, h, _aligned(lo // 2, depth // 2)] = pltpu.bitcast(w[t], I32)
                bulk_s[m, h] = jnp.where(lo > 0, bulk_s[m, h], 0.0) + new[t]

    sub_id = lax.broadcasted_iota(I32, (8, LANES), 0)
    lane_id = lax.broadcasted_iota(I32, (8, LANES), 1)

    def route(part):
        per, half = LANES // seg, d_model // 2
        r = jnp.zeros((8, LANES), F32)
        for j in range(4):
            segs = pl.ds((part * 4 + j) * per, per)
            x = x_s[segs].reshape(LANES, d_model)
            z = _dot_nt(vec_s[:, :half], x[:, :half])
            yield
            z = _dot_nt(vec_s[:, half:], x[:, half:]) + z
            r = jnp.where(sub_id % 4 == j, z[0:1], r)
            g = jnp.broadcast_to(_sigmoid(z)[1:2], (LANES, LANES)).T
            gate_s[segs] = g.reshape(per, seg, LANES)
            yield
        r_s[part] = r

    def reduce_all(op, join, parts):
        return op(op(functools.reduce(join, parts), axis=1, keepdims=True), axis=0, keepdims=True)

    def pick():
        key = [jnp.where(sub_id < 4, r_s[j], r_s[j + 1]) for j in range(0, r_s.shape[0], 2)]
        key = [a.astype(BF16).astype(F32) for a in key]
        key = [jnp.where(a == a, a, -jnp.inf) for a in key]
        tok = [((8 * j + sub_id) * LANES + lane_id).astype(F32) for j in range(len(key))]
        free = tok
        for i in range(TOPK):
            best = reduce_all(jnp.max, jnp.maximum,
                              [jnp.where(f < n_tok, a, -jnp.inf) for a, f in zip(key, free)])
            got = reduce_all(jnp.min, jnp.minimum,
                             [jnp.where(a == best, f, float(n_tok)) for a, f in zip(key, free)])
            free = [jnp.where(t == got, float(n_tok), f) for t, f in zip(tok, free)]
            idx_s[i] = jnp.clip(got.astype(I32)[0, 0], 0, n_tok - 1)
        for i in range(TOPK):
            row, upper = token_row(x_s, i)
            sel_s[i:i + 1] = unpack(row[...], upper)

    def token_row(ref, i):
        t = idx_s[i]
        return ref.bitcast(I32).at[t // seg, pl.ds(t % seg // 2, 1)], t % 2 == 1

    def unpack(words, upper):
        return pltpu.bitcast(jnp.where(upper, words & -65536, words << 16), F32)

    def routed_ffn():
        def chain(lhs, i, j):
            slab, row = ffn_slot(i, j)
            acc = None
            for k in range(0, lhs.shape[1], N_MXU * LANES):
                w = _bf16(stage_words[slab, pl.ds((row + k) // 2, N_MXU * LANES // 2), :])
                part = _dot(lhs[:, k:k + N_MXU * LANES], w)
                acc = part if acc is None else part + acc
                yield acc

        for j in range(n_ft):
            for gate in chain(sel_s, 0, j):
                yield
            for up in chain(sel_s, 1, j):
                yield
            h_s[:, _tile(j)] = gate * _sigmoid(gate) * up
        y = []
        for j in range(n_dt):
            for down in chain(h_s, 2, j):
                yield
            y.append(down)
        h_s[:, :d_model] = jnp.concatenate(y, axis=1)

    def add_row(ref, i, y):
        row, upper = token_row(ref, i)
        words = row[...]
        new = pltpu.bitcast((unpack(words, upper) + y[i:i + 1]).astype(BF16).astype(F32), I32)
        row[...] = jnp.where(
            upper, new | (words & 65535), lax.shift_right_logical(new, 16) | (words & -65536))

    def scatter():
        x_sel = sel_s[...]
        score = jnp.sum(x_sel * vec_s[0:1], axis=-1, keepdims=True).astype(BF16).astype(F32)
        g = _sigmoid(jnp.sum(x_sel * vec_s[1:2], axis=-1, keepdims=True))
        y = h_s[:, :d_model] * _sigmoid(score)
        for i in range(TOPK):
            add_row(x_s, i, y)
            add_row(out_s, i, y * (1.0 - g))

    def mix(s, dst):
        g = jnp.tile(gate_s[s], (1, n_dt))
        out_s[dst] = (g * a_s[...] + (1.0 - g) * x_s[s].astype(F32)).astype(BF16)

    def set_lhs(mem, s, cols):
        lhs = jnp.concatenate([mem, x_s[s, :, cols].astype(F32)[n_mem:]], axis=0)
        lhs_s[:, cols] = pltpu.bitcast(lhs.astype(BF16), I32)

    def segment(s, chained, last=False, side=None):
        skip = n_mem if last else 0
        qi = lax.broadcasted_iota(I32, (rows - skip, rows), 0) + skip
        ki = lax.broadcasted_iota(I32, (rows - skip, rows), 1)
        mask = jnp.logical_or(qi < n_mem, qi >= ki)

        def project(m, h, k0=0, k1=d_model):
            return _dot(_bf16(lhs_s[:, k0:k1]), _bf16(w_s[m, h, k0 // 2:k1 // 2]))

        def all_rows(m, h, y):
            first = bulk_s[m, h, _aligned(s * n_mem, n_mem)]
            return jnp.concatenate([y[:n_mem], first, y[n_mem:]], axis=0)

        def softmax(q, k):
            t = jnp.where(mask, _dot_nt(q[skip:], k.astype(BF16)) * scale, -1e9)
            e = jnp.exp(t - jnp.max(t, axis=-1, keepdims=True))
            total = jnp.sum(e, axis=-1, keepdims=True)
            inv = pltpu.reciprocal(total, approx=True)
            return e, inv * (2.0 - total * inv)

        attended = []
        todo = [(g, j) for g in range(n_heads // N_MXU) for j in range(n_dt)]
        acc = [None] * n_dt

        def attend(probs, v):
            o = [_dot(e, vh.astype(BF16)) * inv for (e, inv), vh in zip(probs, v)]
            attended.append(jnp.concatenate(o, axis=1))
            if side and 1:
                next(side, None)

        def out_proj(count):
            for g, j in [todo.pop(0) for _ in range(count)]:
                w = _bf16(wo_words[j, g * N_MXU * LANES // 2:(g + 1) * N_MXU * LANES // 2])
                part = _dot(attended[g], w)
                acc[j] = part if acc[j] is None else part + acc[j]
                if side and j in [2, 6]:
                    next(side, None)

        n_groups = n_heads // N_MXU
        for g in range(n_groups):
            heads = range(g * N_MXU, (g + 1) * N_MXU)
            if g == 0 and chained:
                half = d_model // 2
                q = [project(0, h, 0, half) for h in heads]
                k = [project(1, h, 0, half) for h in heads]
                q = [project(0, h, half) + y for h, y in zip(heads, q)]
                k = [project(1, h, half) + y for h, y in zip(heads, k)]
            else:
                q = [project(0, h) for h in heads]
                k = [project(1, h) for h in heads]
            if g > 0:
                attend(probs, v)
            v = [all_rows(2, h, project(2, h)) for h in heads]
            probs = [softmax(all_rows(0, h, qh), all_rows(1, h, kh))
                     for h, qh, kh in zip(heads, q, k)]
            if 2 <= g < n_groups - 1:
                out_proj(n_dt)
        out_proj(len(todo) - n_dt - n_dt // 2)
        attend(probs, v)
        out_proj(len(todo))
        for j in range(n_dt):
            if not last:
                set_lhs(acc[j][:n_mem], s + 1, _tile(j))
            a_s[:, _tile(j)] = acc[j][n_mem - skip:]

    for copy in copies(0):
        copy.start()
    a_s[...] = jnp.zeros(a_s.shape, F32)
    out_s[n_seg - 2:n_seg] = jnp.zeros((2, seg, d_model), BF16)

    @pl.loop(0, 2)
    def _(i):
        advance(i, 0, 2)
        bulk(i * LANES, LANES)

    @pl.loop(2, 5)
    def _(i):
        advance(i, 2, 5)
        bulk((i - 1) * 2 * LANES, 2 * LANES)

    vec_s[...] = jnp.zeros(vec_s.shape, F32)
    vec_s[0:1] = wr_s[...].astype(F32).reshape(1, d_model)
    vec_s[1:2] = gw_s[...].astype(F32).reshape(1, d_model)

    @pl.loop(5, 9)
    def _(i):
        advance(i, 5, 9)
        bulk((i - 3) * 4 * LANES, 4 * LANES, route(i - 5))

    advance(9, 9, 10)
    set_lhs(mem0_s[...].astype(F32), 0, slice(None))
    if HEAD:
        pick()
    for s in range(HEAD):
        if s:
            mix(s - 1, s - 1)
        segment(s, s > 0)

    @pl.loop(HEAD, n_seg - TAIL, step=UNROLL)
    def _(s0):
        @pl.when(s0 == HEAD + UNROLL)
        def _():
            for copy in copies(len(batches) - 1):
                copy.start()

        for u in range(UNROLL):
            s = s0 + u
            mix(jnp.maximum(s - 1, 0), jnp.where(s > 0, s - 1, n_seg))
            segment(s, u > 0)

    for copy in copies(len(batches) - 1):
        copy.wait()
    if not HEAD:
        pick()
    ffn = routed_ffn()
    for s in range(n_seg - TAIL, n_seg - 1):
        mix(s - 1, s - 1)
        segment(s, s > n_seg - TAIL, side=ffn if HEAD or s > n_seg - TAIL else None)
    for _ in ffn:
        pass
    scatter()
    out_copy(0, n_seg - 2).start()
    pl.semaphore_signal(order_sem)
    pl.semaphore_wait(order_sem)
    mix(n_seg - 2, n_seg - 2)
    segment(n_seg - 1, False, last=True)
    mix(n_seg - 1, n_seg - 1)
    out_copy(n_seg - 2, n_seg).start()
    out_copy(0, n_seg - 2).wait()
    out_copy(n_seg - 2, n_seg).wait()


def pallas_gated_mix__memory_aug_recurrent_mem_tr__moe_arch_mod__prompt_kernel(
    A_x, A_mem0, A_Wq, A_Wk, A_Wv, A_Wo, A_seg_len,
    B_x, B_w_r, B_w_gate, B_w_up, B_w_down, gate_w,
):
    del B_x
    seg = int(A_seg_len)
    batch, n_tok, d_model = A_x.shape
    _, n_heads, d_head = A_Wq.shape
    n_mem = A_mem0.shape[1]
    d_ffn = B_w_gate.shape[1]
    n_seg, n_dt = n_tok // seg, d_model // LANES
    assert (batch, n_seg, seg, d_model, n_mem, d_head) == (1, 64, 32, 1024, 8, LANES)

    hbm = pl.BlockSpec(memory_space=pl.ANY)
    out = pl.pallas_call(
        _kernel,
        out_shape=jax.ShapeDtypeStruct((n_seg, seg, d_model), BF16),
        in_specs=[hbm] * 11,
        out_specs=hbm,
        scratch_shapes=[
            pltpu.VMEM((3, n_heads, d_model // 2, LANES), I32),
            pltpu.VMEM((n_dt, n_heads * LANES, LANES), BF16),
            pltpu.VMEM((3 * n_dt, LANES * n_heads, LANES), BF16),
            pltpu.VMEM((n_dt, n_seg, n_mem, LANES), BF16),
            pltpu.VMEM((3, n_heads, n_seg * n_mem, LANES), F32),
            pltpu.VMEM((n_seg, seg, d_model), BF16),
            pltpu.VMEM((seg // 2, d_model), I32),
            pltpu.VMEM((seg, d_model), F32),
            pltpu.VMEM((n_seg, seg, LANES), F32),
            pltpu.VMEM((n_seg + 1, seg, d_model), BF16),
            pltpu.VMEM((n_mem, d_model), BF16),
            pltpu.VMEM((d_model,), BF16),
            pltpu.VMEM((d_model,), BF16),
            pltpu.VMEM((8, d_model), F32),
            pltpu.VMEM((4, 8, LANES), F32),
            pltpu.VMEM((TOPK, d_model), F32),
            pltpu.VMEM((TOPK, d_ffn), F32),
            pltpu.SMEM((TOPK,), I32),
            pltpu.SemaphoreType.DMA((12,)),
            pltpu.SemaphoreType.REGULAR(()),
        ],
        compiler_params=pltpu.CompilerParams(vmem_limit_bytes=110 * 1024 * 1024),
    )(
        A_x.reshape(n_seg, seg, d_model),
        A_mem0.reshape(n_mem, d_model),
        A_Wq.reshape(n_dt, LANES * n_heads, d_head),
        A_Wk.reshape(n_dt, LANES * n_heads, d_head),
        A_Wv.reshape(n_dt, LANES * n_heads, d_head),
        A_Wo.reshape(n_heads * d_head, d_model),
        B_w_r,
        B_w_gate,
        B_w_up,
        B_w_down,
        gate_w,
    )
    return out.reshape(batch, n_tok, d_model)
```

```python
import functools

import jax
import jax.numpy as jnp
from jax import lax
from jax.experimental import pallas as pl
from jax.experimental.pallas import tpu as pltpu

F32, BF16, I32 = jnp.float32, jnp.bfloat16, jnp.int32

LANES = 128
N_MXU = 4
TOPK = 8
UNROLL = 4
TAIL = 12


def _dot(a, b):
    return lax.dot_general(a, b, (((1,), (0,)), ((), ())), preferred_element_type=F32)


def _dot_nt(a, b):
    return lax.dot_general(a, b, (((1,), (1,)), ((), ())), preferred_element_type=F32)


def _bf16(words):
    return pltpu.bitcast(words, BF16)


def _aligned(start, size):
    return pl.ds(start if isinstance(start, int) else pl.multiple_of(start, size), size)


def _tile(j):
    return slice(j * LANES, (j + 1) * LANES)


def _sigmoid(z):
    return 1.0 / (1.0 + jnp.exp(-z))


def _kernel(
    x_hbm, mem0_hbm, wq_hbm, wk_hbm, wv_hbm, wo_hbm, wr_hbm, wg_hbm, wu_hbm, wd_hbm, gw_hbm,
    out_hbm,
    w_s, wo_s, stage_s, xh_s, bulk_s, x_s, lhs_s, a_s, gate_s, out_s,
    mem0_s, wr_s, gw_s, vec_s, r_s, sel_s, h_s, idx_s, sem, order_sem,
):
    n_seg, seg, d_model = x_hbm.shape
    n_tok = n_seg * seg
    n_heads = w_s.shape[1]
    n_mem = mem0_hbm.shape[0]
    d_ffn = wd_hbm.shape[0]
    n_dt, n_ft = d_model // LANES, d_ffn // LANES
    rows = n_mem + seg
    pairs = n_heads // 2
    scale = LANES ** -0.5

    def weight_copy(m, lo, hi):
        return (wq_hbm, wk_hbm, wv_hbm)[m].at[lo:hi], stage_s.at[m * n_dt + lo:m * n_dt + hi]

    def part_copy(j, lo, hi):
        part = pl.ds(lo * n_heads, (hi - lo) * n_heads)
        return wq_hbm.at[j, part], stage_s.at[j, part]

    def head_copies(lo, hi):
        return [(x_hbm.at[:, :n_mem, _tile(j)], xh_s.at[j]) for j in range(lo, hi)]

    def x_copy(i):
        segs = pl.ds(i * n_seg // 4, n_seg // 4)
        return x_hbm.at[segs], x_s.at[segs]

    def wo_copies(lo, hi):
        return [(wo_hbm.at[:, _tile(j)], wo_s.at[j]) for j in range(lo, hi)]

    def ffn_slot(i, j):
        if i == 2:
            return 2 * n_dt + j, 0
        slab, k = divmod(i * n_ft + j, LANES * n_heads // d_model)
        return slab, k * d_model

    def ffn_copies(i, w_hbm):
        depth, width = w_hbm.shape
        slots = [ffn_slot(i, j) for j in range(width // LANES)]
        return [(w_hbm.at[:, _tile(j)], stage_s.at[slab, pl.ds(row, depth)])
                for j, (slab, row) in enumerate(slots)]

    batches = [
        [part_copy(0, 0, 64)] + head_copies(0, 1) + [part_copy(0, 64, 128)],
        [weight_copy(0, 1, 2), part_copy(2, 0, 64)] + head_copies(1, 2),
        [part_copy(2, 64, 128), weight_copy(0, 3, 4)] + head_copies(2, 4),
        [weight_copy(0, 4, 7)] + head_copies(4, 6),
        [weight_copy(0, 7, 8), weight_copy(1, 0, 2)] + head_copies(6, 8)
        + [(mem0_hbm, mem0_s), (wr_hbm, wr_s), (gw_hbm, gw_s)],
        [weight_copy(1, 2, 4), x_copy(0)],
        [weight_copy(1, 4, 8), x_copy(1)],
        [weight_copy(2, 0, 4), x_copy(2)] + wo_copies(0, 2),
        [weight_copy(2, 4, 8), x_copy(3)] + wo_copies(2, 3),
        wo_copies(3, n_dt),
        ffn_copies(0, wg_hbm) + ffn_copies(1, wu_hbm) + ffn_copies(2, wd_hbm),
    ]

    def copies(i):
        return [pltpu.make_async_copy(src, dst, sem.at[i]) for src, dst in batches[i]]

    def advance(i, lo, hi):
        for c in range(lo, hi):
            @pl.when(i == c)
            def _(c=c):
                *most, rest = copies(c)
                for copy in most:
                    copy.wait()
                for copy in copies(c + 1) if c + 2 < len(batches) else ():
                    copy.start()
                rest.wait()

    def out_copy(lo, hi):
        return pltpu.make_async_copy(out_s.at[lo:hi], out_hbm.at[lo:hi], sem.at[len(batches)])

    stage_words = stage_s.bitcast(I32)
    wo_words = wo_s.bitcast(I32)

    def bulk(k0, depth, side=()):
        m, lo = k0 // d_model, k0 % d_model
        side = iter(side)

        def xh(a, b):
            return jnp.concatenate(
                [xh_s[lo // LANES + j].reshape(n_seg * n_mem, LANES)
                 for j in range(a // LANES, b // LANES)], axis=1)

        for p in range(pairs):
            words = jnp.concatenate(
                [stage_words[k0 // LANES + j, pl.ds(p, LANES, stride=pairs), :]
                 for j in range(depth // LANES)], axis=0)
            w = [pltpu.bitcast(half, F32).astype(BF16) for half in (words << 16, words & -65536)]
            if p == 0 or depth < N_MXU * LANES:
                both = None
                for a in range(0, depth, 2 * LANES):
                    b = min(a + 2 * LANES, depth)
                    part = _dot(xh(a, b), jnp.concatenate(w, axis=1)[a:b])
                    both = part if both is None else part + both
                new = [both[:, _tile(t)] for t in range(2)]
            else:
                new = [_dot(xh(0, depth), w[0])]
                next(side, None)
                new.append(_dot(xh(0, depth), w[1]))
            for t in range(2):
                h = 2 * p + t
                w_s[m, h, _aligned(lo // 2, depth // 2)] = pltpu.bitcast(w[t], I32)
                bulk_s[m, h] = jnp.where(lo > 0, bulk_s[m, h], 0.0) + new[t]

    sub_id = lax.broadcasted_iota(I32, (8, LANES), 0)
    lane_id = lax.broadcasted_iota(I32, (8, LANES), 1)

    def route(part):
        per, half = LANES // seg, d_model // 2
        r = jnp.zeros((8, LANES), F32)
        for j in range(4):
            segs = pl.ds((part * 4 + j) * per, per)
            x = x_s[segs].reshape(LANES, d_model)
            z = _dot_nt(vec_s[:, :half], x[:, :half])
            yield
            z = _dot_nt(vec_s[:, half:], x[:, half:]) + z
            r = jnp.where(sub_id % 4 == j, z[0:1], r)
            g = jnp.broadcast_to(_sigmoid(z)[1:2], (LANES, LANES)).T
            gate_s[segs] = g.reshape(per, seg, LANES)
            yield
        r_s[part] = r

    def reduce_all(op, join, parts):
        return op(op(functools.reduce(join, parts), axis=1, keepdims=True), axis=0, keepdims=True)

    def pick():
        key = [jnp.where(sub_id < 4, r_s[j], r_s[j + 1]) for j in range(0, r_s.shape[0], 2)]
        key = [a.astype(BF16).astype(F32) for a in key]
        key = [jnp.where(a == a, a, -jnp.inf) for a in key]
        tok = [((8 * j + sub_id) * LANES + lane_id).astype(F32) for j in range(len(key))]
        free = tok
        for i in range(TOPK):
            best = reduce_all(jnp.max, jnp.maximum,
                              [jnp.where(f < n_tok, a, -jnp.inf) for a, f in zip(key, free)])
            got = reduce_all(jnp.min, jnp.minimum,
                             [jnp.where(a == best, f, float(n_tok)) for a, f in zip(key, free)])
            free = [jnp.where(t == got, float(n_tok), f) for t, f in zip(tok, free)]
            idx_s[i] = jnp.clip(got.astype(I32)[0, 0], 0, n_tok - 1)
        for i in range(TOPK):
            row, upper = token_row(x_s, i)
            sel_s[i:i + 1] = unpack(row[...], upper)

    def token_row(ref, i):
        t = idx_s[i]
        return ref.bitcast(I32).at[t // seg, pl.ds(t % seg // 2, 1)], t % 2 == 1

    def unpack(words, upper):
        return pltpu.bitcast(jnp.where(upper, words & -65536, words << 16), F32)

    def routed_ffn():
        def chain(lhs, i, j):
            slab, row = ffn_slot(i, j)
            acc = None
            for k in range(0, lhs.shape[1], N_MXU * LANES):
                w = _bf16(stage_words[slab, pl.ds((row + k) // 2, N_MXU * LANES // 2), :])
                part = _dot(lhs[:, k:k + N_MXU * LANES], w)
                acc = part if acc is None else part + acc
                yield acc

        for j in range(n_ft):
            for gate in chain(sel_s, 0, j):
                yield
            for up in chain(sel_s, 1, j):
                yield
            h_s[:, _tile(j)] = gate * _sigmoid(gate) * up
        y = []
        for j in range(n_dt):
            for down in chain(h_s, 2, j):
                yield
            y.append(down)
        h_s[:, :d_model] = jnp.concatenate(y, axis=1)

    def add_row(ref, i, y):
        row, upper = token_row(ref, i)
        words = row[...]
        new = pltpu.bitcast((unpack(words, upper) + y[i:i + 1]).astype(BF16).astype(F32), I32)
        row[...] = jnp.where(
            upper, new | (words & 65535), lax.shift_right_logical(new, 16) | (words & -65536))

    def scatter():
        x_sel = sel_s[...]
        score = jnp.sum(x_sel * vec_s[0:1], axis=-1, keepdims=True).astype(BF16).astype(F32)
        g = _sigmoid(jnp.sum(x_sel * vec_s[1:2], axis=-1, keepdims=True))
        y = h_s[:, :d_model] * _sigmoid(score)
        for i in range(TOPK):
            add_row(x_s, i, y)
            add_row(out_s, i, y * (1.0 - g))

    def mix(s, dst):
        g = jnp.tile(gate_s[s], (1, n_dt))
        out_s[dst] = (g * a_s[...] + (1.0 - g) * x_s[s].astype(F32)).astype(BF16)

    def set_lhs(mem, s, cols):
        lhs = jnp.concatenate([mem, x_s[s, :, cols].astype(F32)[n_mem:]], axis=0)
        lhs_s[:, cols] = pltpu.bitcast(lhs.astype(BF16), I32)

    def segment(s, chained, last=False, side=None):
        skip = n_mem if last else 0
        qi = lax.broadcasted_iota(I32, (rows - skip, rows), 0) + skip
        ki = lax.broadcasted_iota(I32, (rows - skip, rows), 1)
        mask = jnp.logical_or(qi < n_mem, qi >= ki)

        def project(m, h, k0=0, k1=d_model):
            return _dot(_bf16(lhs_s[:, k0:k1]), _bf16(w_s[m, h, k0 // 2:k1 // 2]))

        def all_rows(m, h, y):
            first = bulk_s[m, h, _aligned(s * n_mem, n_mem)]
            return jnp.concatenate([y[:n_mem], first, y[n_mem:]], axis=0)

        def softmax(q, k):
            t = jnp.where(mask, _dot_nt(q[skip:], k.astype(BF16)) * scale, -1e9)
            e = jnp.exp(t - jnp.max(t, axis=-1, keepdims=True))
            total = jnp.sum(e, axis=-1, keepdims=True)
            inv = pltpu.reciprocal(total, approx=True)
            return e, inv * (2.0 - total * inv)

        attended = []
        todo = [(g, j) for g in range(n_heads // N_MXU) for j in range(n_dt)]
        acc = [None] * n_dt

        def attend(probs, v):
            o = [_dot(e, vh.astype(BF16)) * inv for (e, inv), vh in zip(probs, v)]
            attended.append(jnp.concatenate(o, axis=1))

        def out_proj(count):
            for g, j in [todo.pop(0) for _ in range(count)]:
                w = _bf16(wo_words[j, g * N_MXU * LANES // 2:(g + 1) * N_MXU * LANES // 2])
                part = _dot(attended[g], w)
                acc[j] = part if acc[j] is None else part + acc[j]
                if side and j in (0, 3):
                    next(side, None)

        n_groups = n_heads // N_MXU
        for g in range(n_groups):
            heads = range(g * N_MXU, (g + 1) * N_MXU)
            if g == 0 and chained:
                half = d_model // 2
                q = [project(0, h, 0, half) for h in heads]
                k = [project(1, h, 0, half) for h in heads]
                q = [project(0, h, half) + y for h, y in zip(heads, q)]
                k = [project(1, h, half) + y for h, y in zip(heads, k)]
            else:
                q = [project(0, h) for h in heads]
                k = [project(1, h) for h in heads]
            if g > 0:
                attend(probs, v)
            v = [all_rows(2, h, project(2, h)) for h in heads]
            probs = [softmax(all_rows(0, h, qh), all_rows(1, h, kh))
                     for h, qh, kh in zip(heads, q, k)]
            if 2 <= g < n_groups - 1:
                out_proj(n_dt)
        out_proj(len(todo) - n_dt - n_dt // 2)
        attend(probs, v)
        out_proj(len(todo))
        for j in range(n_dt):
            if not last:
                set_lhs(acc[j][:n_mem], s + 1, _tile(j))
            a_s[:, _tile(j)] = acc[j][n_mem - skip:]

    for copy in copies(0):
        copy.start()
    a_s[...] = jnp.zeros(a_s.shape, F32)
    out_s[n_seg - 1] = jnp.zeros((seg, d_model), BF16)

    @pl.loop(0, 2)
    def _(i):
        advance(i, 0, 2)
        bulk(i * LANES, LANES)

    @pl.loop(2, 5)
    def _(i):
        advance(i, 2, 5)
        bulk((i - 1) * 2 * LANES, 2 * LANES)

    vec_s[...] = jnp.zeros(vec_s.shape, F32)
    vec_s[0:1] = wr_s[...].astype(F32).reshape(1, d_model)
    vec_s[1:2] = gw_s[...].astype(F32).reshape(1, d_model)

    @pl.loop(5, 9)
    def _(i):
        advance(i, 5, 9)
        bulk((i - 3) * 4 * LANES, 4 * LANES, route(i - 5))

    advance(9, 9, 10)
    set_lhs(mem0_s[...].astype(F32), 0, slice(None))

    @pl.loop(0, n_seg - TAIL, step=UNROLL)
    def _(s0):
        @pl.when(s0 == UNROLL)
        def _():
            for copy in copies(len(batches) - 1):
                copy.start()

        for u in range(UNROLL):
            s = s0 + u
            mix(jnp.maximum(s - 1, 0), jnp.where(s > 0, s - 1, n_seg))
            segment(s, u > 0)

    for copy in copies(len(batches) - 1):
        copy.wait()
    pick()
    ffn = routed_ffn()
    for s in range(n_seg - TAIL, n_seg - 1):
        mix(s - 1, s - 1)
        segment(s, s > n_seg - TAIL, side=ffn if s > n_seg - TAIL else None)
    for _ in ffn:
        pass
    mix(n_seg - 2, n_seg - 2)
    scatter()
    out_copy(0, n_seg - 1).start()
    pl.semaphore_signal(order_sem)
    pl.semaphore_wait(order_sem)
    segment(n_seg - 1, False, last=True)
    mix(n_seg - 1, n_seg - 1)
    out_copy(n_seg - 1, n_seg).start()
    out_copy(0, n_seg - 1).wait()
    out_copy(n_seg - 1, n_seg).wait()


def pallas_gated_mix__memory_aug_recurrent_mem_tr__moe_arch_mod__prompt_kernel(
    A_x, A_mem0, A_Wq, A_Wk, A_Wv, A_Wo, A_seg_len,
    B_x, B_w_r, B_w_gate, B_w_up, B_w_down, gate_w,
):
    del B_x
    seg = int(A_seg_len)
    batch, n_tok, d_model = A_x.shape
    _, n_heads, d_head = A_Wq.shape
    n_mem = A_mem0.shape[1]
    d_ffn = B_w_gate.shape[1]
    n_seg, n_dt = n_tok // seg, d_model // LANES
    assert (batch, n_seg, seg, d_model, n_mem, d_head) == (1, 64, 32, 1024, 8, LANES)

    hbm = pl.BlockSpec(memory_space=pl.ANY)
    out = pl.pallas_call(
        _kernel,
        out_shape=jax.ShapeDtypeStruct((n_seg, seg, d_model), BF16),
        in_specs=[hbm] * 11,
        out_specs=hbm,
        scratch_shapes=[
            pltpu.VMEM((3, n_heads, d_model // 2, LANES), I32),
            pltpu.VMEM((n_dt, n_heads * LANES, LANES), BF16),
            pltpu.VMEM((3 * n_dt, LANES * n_heads, LANES), BF16),
            pltpu.VMEM((n_dt, n_seg, n_mem, LANES), BF16),
            pltpu.VMEM((3, n_heads, n_seg * n_mem, LANES), F32),
            pltpu.VMEM((n_seg, seg, d_model), BF16),
            pltpu.VMEM((seg // 2, d_model), I32),
            pltpu.VMEM((seg, d_model), F32),
            pltpu.VMEM((n_seg, seg, LANES), F32),
            pltpu.VMEM((n_seg + 1, seg, d_model), BF16),
            pltpu.VMEM((n_mem, d_model), BF16),
            pltpu.VMEM((d_model,), BF16),
            pltpu.VMEM((d_model,), BF16),
            pltpu.VMEM((8, d_model), F32),
            pltpu.VMEM((4, 8, LANES), F32),
            pltpu.VMEM((TOPK, d_model), F32),
            pltpu.VMEM((TOPK, d_ffn), F32),
            pltpu.SMEM((TOPK,), I32),
            pltpu.SemaphoreType.DMA((12,)),
            pltpu.SemaphoreType.REGULAR(()),
        ],
        compiler_params=pltpu.CompilerParams(vmem_limit_bytes=110 * 1024 * 1024),
    )(
        A_x.reshape(n_seg, seg, d_model),
        A_mem0.reshape(n_mem, d_model),
        A_Wq.reshape(n_dt, LANES * n_heads, d_head),
        A_Wk.reshape(n_dt, LANES * n_heads, d_head),
        A_Wv.reshape(n_dt, LANES * n_heads, d_head),
        A_Wo.reshape(n_heads * d_head, d_model),
        B_w_r,
        B_w_gate,
        B_w_up,
        B_w_down,
        gate_w,
    )
    return out.reshape(batch, n_tok, d_model)
```

```python
import functools

import jax
import jax.numpy as jnp
from jax import lax
from jax.experimental import pallas as pl
from jax.experimental.pallas import tpu as pltpu

F32, BF16, I32 = jnp.float32, jnp.bfloat16, jnp.int32

LANES = 128
N_MXU = 4
TOPK = 8
UNROLL = 4
TAIL = 12


def _dot(a, b):
    return lax.dot_general(a, b, (((1,), (0,)), ((), ())), preferred_element_type=F32)


def _dot_nt(a, b):
    return lax.dot_general(a, b, (((1,), (1,)), ((), ())), preferred_element_type=F32)


def _bf16(words):
    return pltpu.bitcast(words, BF16)


def _aligned(start, size):
    return pl.ds(start if isinstance(start, int) else pl.multiple_of(start, size), size)


def _tile(j):
    return slice(j * LANES, (j + 1) * LANES)


def _sigmoid(z):
    return 1.0 / (1.0 + jnp.exp(-z))


def _kernel(
    x_hbm, mem0_hbm, wq_hbm, wk_hbm, wv_hbm, wo_hbm, wr_hbm, wg_hbm, wu_hbm, wd_hbm, gw_hbm,
    out_hbm,
    w_s, wo_s, stage_s, xh_s, bulk_s, x_s, lhs_s, a_s, gate_s, out_s,
    mem0_s, wr_s, gw_s, vec_s, r_s, sel_s, h_s, idx_s, sem, order_sem,
):
    n_seg, seg, d_model = x_hbm.shape
    n_tok = n_seg * seg
    n_heads = w_s.shape[1]
    n_mem = mem0_hbm.shape[0]
    d_ffn = wd_hbm.shape[0]
    n_dt, n_ft = d_model // LANES, d_ffn // LANES
    rows = n_mem + seg
    pairs = n_heads // 2
    scale = LANES ** -0.5

    def weight_copy(m, lo, hi):
        return (wq_hbm, wk_hbm, wv_hbm)[m].at[lo:hi], stage_s.at[m * n_dt + lo:m * n_dt + hi]

    def part_copy(j, lo, hi):
        part = pl.ds(lo * n_heads, (hi - lo) * n_heads)
        return wq_hbm.at[j, part], stage_s.at[j, part]

    def head_copies(lo, hi):
        return [(x_hbm.at[:, :n_mem, _tile(j)], xh_s.at[j]) for j in range(lo, hi)]

    def x_copy(i):
        segs = pl.ds(i * n_seg // 4, n_seg // 4)
        return x_hbm.at[segs], x_s.at[segs]

    def wo_copies(lo, hi):
        return [(wo_hbm.at[:, _tile(j)], wo_s.at[j]) for j in range(lo, hi)]

    def ffn_slot(i, j):
        if i == 2:
            return 2 * n_dt + j, 0
        slab, k = divmod(i * n_ft + j, LANES * n_heads // d_model)
        return slab, k * d_model

    def ffn_copies(i, w_hbm):
        depth, width = w_hbm.shape
        slots = [ffn_slot(i, j) for j in range(width // LANES)]
        return [(w_hbm.at[:, _tile(j)], stage_s.at[slab, pl.ds(row, depth)])
                for j, (slab, row) in enumerate(slots)]

    batches = [
        [part_copy(0, 0, 32)] + head_copies(0, 1) + [part_copy(0, 32, 128)],
        [weight_copy(0, 1, 2), part_copy(2, 0, 64)] + head_copies(1, 2),
        [part_copy(2, 64, 128), weight_copy(0, 3, 4)] + head_copies(2, 4),
        [weight_copy(0, 4, 7)] + head_copies(4, 6),
        [weight_copy(0, 7, 8), weight_copy(1, 0, 2)] + head_copies(6, 8)
        + [(mem0_hbm, mem0_s), (wr_hbm, wr_s), (gw_hbm, gw_s)],
        [weight_copy(1, 2, 4), x_copy(0)],
        [weight_copy(1, 4, 8), x_copy(1)],
        [weight_copy(2, 0, 4), x_copy(2)] + wo_copies(0, 2),
        [weight_copy(2, 4, 8), x_copy(3)] + wo_copies(2, 3),
        wo_copies(3, n_dt),
        ffn_copies(0, wg_hbm) + ffn_copies(1, wu_hbm) + ffn_copies(2, wd_hbm),
    ]

    def copies(i):
        return [pltpu.make_async_copy(src, dst, sem.at[i]) for src, dst in batches[i]]

    def advance(i, lo, hi):
        for c in range(lo, hi):
            @pl.when(i == c)
            def _(c=c):
                *most, rest = copies(c)
                for copy in most:
                    copy.wait()
                for copy in copies(c + 1) if c + 2 < len(batches) else ():
                    copy.start()
                rest.wait()

    def out_copy(lo, hi):
        return pltpu.make_async_copy(out_s.at[lo:hi], out_hbm.at[lo:hi], sem.at[len(batches)])

    stage_words, wo_words = stage_s.bitcast(I32), wo_s.bitcast(I32)

    def bulk(k0, depth, side=()):
        m, lo = k0 // d_model, k0 % d_model
        side = iter(side)

        def xh(a, b):
            return jnp.concatenate(
                [xh_s[lo // LANES + j].reshape(n_seg * n_mem, LANES)
                 for j in range(a // LANES, b // LANES)], axis=1)

        for p in range(pairs):
            words = jnp.concatenate(
                [stage_words[k0 // LANES + j, pl.ds(p, LANES, stride=pairs), :]
                 for j in range(depth // LANES)], axis=0)
            w = [pltpu.bitcast(half, F32).astype(BF16) for half in (words << 16, words & -65536)]
            if p == 0 or depth < N_MXU * LANES:
                both = None
                for a in range(0, depth, 2 * LANES):
                    b = min(a + 2 * LANES, depth)
                    part = _dot(xh(a, b), jnp.concatenate(w, axis=1)[a:b])
                    both = part if both is None else part + both
                new = [both[:, _tile(t)] for t in range(2)]
            else:
                new = [_dot(xh(0, depth), w[0])]
                next(side, None)
                new.append(_dot(xh(0, depth), w[1]))
            for t in range(2):
                h = 2 * p + t
                w_s[m, h, _aligned(lo // 2, depth // 2)] = pltpu.bitcast(w[t], I32)
                bulk_s[m, h] = jnp.where(lo > 0, bulk_s[m, h], 0.0) + new[t]

    sub_id = lax.broadcasted_iota(I32, (8, LANES), 0)
    lane_id = lax.broadcasted_iota(I32, (8, LANES), 1)

    def route(part):
        per, half = LANES // seg, d_model // 2
        r = jnp.zeros((8, LANES), F32)
        for j in range(4):
            segs = pl.ds((part * 4 + j) * per, per)
            x = x_s[segs].reshape(LANES, d_model)
            z = _dot_nt(vec_s[:, :half], x[:, :half])
            yield
            z = _dot_nt(vec_s[:, half:], x[:, half:]) + z
            r = jnp.where(sub_id % 4 == j, z[0:1], r)
            g = jnp.broadcast_to(_sigmoid(z)[1:2], (LANES, LANES)).T
            gate_s[segs] = g.reshape(per, seg, LANES)
            yield
        r_s[part] = r

    def reduce_all(op, join, parts):
        return op(op(functools.reduce(join, parts), axis=1, keepdims=True), axis=0, keepdims=True)

    def pick():
        key = [jnp.where(sub_id < 4, r_s[j], r_s[j + 1]) for j in range(0, r_s.shape[0], 2)]
        key = [a.astype(BF16).astype(F32) for a in key]
        key = [jnp.where(a == a, a, -jnp.inf) for a in key]
        tok = [((8 * j + sub_id) * LANES + lane_id).astype(F32) for j in range(len(key))]
        free = tok
        for i in range(TOPK):
            best = reduce_all(jnp.max, jnp.maximum,
                              [jnp.where(f < n_tok, a, -jnp.inf) for a, f in zip(key, free)])
            got = reduce_all(jnp.min, jnp.minimum,
                             [jnp.where(a == best, f, float(n_tok)) for a, f in zip(key, free)])
            free = [jnp.where(t == got, float(n_tok), f) for t, f in zip(tok, free)]
            idx_s[i] = jnp.clip(got.astype(I32)[0, 0], 0, n_tok - 1)
        for i in range(TOPK):
            sel_s[i:i + 1] = unpack(token_words(x_s, i)[...], i)

    def token_words(ref, i):
        return ref.bitcast(I32).at[idx_s[i] // seg, pl.ds(idx_s[i] % seg // 2, 1)]

    def unpack(words, i):
        return pltpu.bitcast(jnp.where(idx_s[i] % 2 == 1, words & -65536, words << 16), F32)

    def routed_ffn():
        def chain(lhs, i, j):
            slab, row = ffn_slot(i, j)
            acc = None
            for k in range(0, lhs.shape[1], N_MXU * LANES):
                w = _bf16(stage_words[slab, pl.ds((row + k) // 2, N_MXU * LANES // 2), :])
                part = _dot(lhs[:, k:k + N_MXU * LANES], w)
                acc = part if acc is None else part + acc
                yield acc

        for j in range(n_ft):
            for gate in chain(sel_s, 0, j):
                yield
            for up in chain(sel_s, 1, j):
                yield
            h_s[:, _tile(j)] = gate * _sigmoid(gate) * up
        y = []
        for j in range(n_dt):
            for down in chain(h_s, 2, j):
                yield
            y.append(down)
        h_s[:, :d_model] = jnp.concatenate(y, axis=1)

    def scatter():
        x_sel = sel_s[...]
        score = jnp.sum(x_sel * vec_s[0:1], axis=-1, keepdims=True).astype(BF16).astype(F32)
        g = _sigmoid(jnp.sum(x_sel * vec_s[1:2], axis=-1, keepdims=True))
        y = h_s[:, :d_model] * (_sigmoid(score) * (1.0 - g))
        for i in range(TOPK):
            row = token_words(out_s, i)
            words = row[...]
            new = pltpu.bitcast((unpack(words, i) + y[i:i + 1]).astype(BF16).astype(F32), I32)
            row[...] = jnp.where(idx_s[i] % 2 == 1, new | (words & 65535),
                                 lax.shift_right_logical(new, 16) | (words & -65536))

    def mix(s, dst, scattered=False):
        g = jnp.tile(gate_s[s], (1, n_dt))
        out = g * a_s[...] + (1.0 - g) * x_s[s].astype(F32)
        if scattered:
            out = out + out_s[dst].astype(F32)
        out_s[dst] = out.astype(BF16)

    def set_lhs(mem, s, cols):
        lhs = jnp.concatenate([mem, x_s[s, :, cols].astype(F32)[n_mem:]], axis=0)
        lhs_s[:, cols] = pltpu.bitcast(lhs.astype(BF16), I32)

    def segment(s, chained, last=False, side=None):
        skip = n_mem if last else 0
        qi = lax.broadcasted_iota(I32, (rows - skip, rows), 0) + skip
        ki = lax.broadcasted_iota(I32, (rows - skip, rows), 1)
        mask = jnp.logical_or(qi < n_mem, qi >= ki)

        def project(m, h, k0=0, k1=d_model):
            return _dot(_bf16(lhs_s[:, k0:k1]), _bf16(w_s[m, h, k0 // 2:k1 // 2]))

        def all_rows(m, h, y):
            first = bulk_s[m, h, _aligned(s * n_mem, n_mem)]
            return jnp.concatenate([y[:n_mem], first, y[n_mem:]], axis=0)

        def softmax(q, k):
            t = jnp.where(mask, _dot_nt(q[skip:], k.astype(BF16)) * scale, -1e9)
            e = jnp.exp(t - jnp.max(t, axis=-1, keepdims=True))
            total = jnp.sum(e, axis=-1, keepdims=True)
            inv = pltpu.reciprocal(total, approx=True)
            return e, inv * (2.0 - total * inv)

        attended = []
        todo = [(g, j) for g in range(n_heads // N_MXU) for j in range(n_dt)]
        acc = [None] * n_dt

        def attend(probs, v):
            o = [_dot(e, vh.astype(BF16)) * inv for (e, inv), vh in zip(probs, v)]
            attended.append(jnp.concatenate(o, axis=1))

        def out_proj(count):
            for g, j in [todo.pop(0) for _ in range(count)]:
                w = _bf16(wo_words[j, g * N_MXU * LANES // 2:(g + 1) * N_MXU * LANES // 2])
                part = _dot(attended[g], w)
                acc[j] = part if acc[j] is None else part + acc[j]
                if side and j in (0, 3):
                    next(side, None)

        n_groups = n_heads // N_MXU
        for g in range(n_groups):
            heads = range(g * N_MXU, (g + 1) * N_MXU)
            if g == 0 and chained:
                half = d_model // 2
                q = [project(0, h, 0, half) for h in heads]
                k = [project(1, h, 0, half) for h in heads]
                q = [project(0, h, half) + y for h, y in zip(heads, q)]
                k = [project(1, h, half) + y for h, y in zip(heads, k)]
            else:
                q = [project(0, h) for h in heads]
                k = [project(1, h) for h in heads]
            if g > 0:
                attend(probs, v)
            v = [all_rows(2, h, project(2, h)) for h in heads]
            probs = [softmax(all_rows(0, h, qh), all_rows(1, h, kh))
                     for h, qh, kh in zip(heads, q, k)]
            if 2 <= g < n_groups - 1:
                out_proj(n_dt)
        out_proj(len(todo) - n_dt - n_dt // 2)
        attend(probs, v)
        out_proj(len(todo))
        for j in range(n_dt):
            if not last:
                set_lhs(acc[j][:n_mem], s + 1, _tile(j))
            a_s[:, _tile(j)] = acc[j][n_mem - skip:]

    for copy in copies(0):
        copy.start()
    a_s[...] = jnp.zeros(a_s.shape, F32)
    out_s[n_seg - 1] = jnp.zeros((seg, d_model), BF16)

    @pl.loop(0, 2)
    def _(i):
        advance(i, 0, 2)
        bulk(i * LANES, LANES)

    @pl.loop(2, 5)
    def _(i):
        advance(i, 2, 5)
        bulk((i - 1) * 2 * LANES, 2 * LANES)

    vec_s[...] = jnp.zeros(vec_s.shape, F32)
    vec_s[0:1] = wr_s[...].astype(F32).reshape(1, d_model)
    vec_s[1:2] = gw_s[...].astype(F32).reshape(1, d_model)

    @pl.loop(5, 9)
    def _(i):
        advance(i, 5, 9)
        bulk((i - 3) * 4 * LANES, 4 * LANES, route(i - 5))

    advance(9, 9, 10)
    set_lhs(mem0_s[...].astype(F32), 0, slice(None))

    @pl.loop(0, n_seg - TAIL, step=UNROLL)
    def _(s0):
        @pl.when(s0 == UNROLL)
        def _():
            for copy in copies(len(batches) - 1):
                copy.start()

        for u in range(UNROLL):
            s = s0 + u
            mix(jnp.maximum(s - 1, 0), jnp.where(s > 0, s - 1, n_seg))
            segment(s, u > 0)

    for copy in copies(len(batches) - 1):
        copy.wait()
    pick()
    ffn = routed_ffn()
    for s in range(n_seg - TAIL, n_seg - 1):
        mix(s - 1, s - 1)
        segment(s, s > n_seg - TAIL, side=ffn if s > n_seg - TAIL else None)
    for _ in ffn:
        pass
    mix(n_seg - 2, n_seg - 2)
    scatter()
    out_copy(0, n_seg - 1).start()
    pl.semaphore_signal(order_sem)
    pl.semaphore_wait(order_sem)
    segment(n_seg - 1, False, last=True)
    mix(n_seg - 1, n_seg - 1, scattered=True)
    out_copy(n_seg - 1, n_seg).start()
    out_copy(0, n_seg - 1).wait()
    out_copy(n_seg - 1, n_seg).wait()


def pallas_gated_mix__memory_aug_recurrent_mem_tr__moe_arch_mod__prompt_kernel(
    A_x, A_mem0, A_Wq, A_Wk, A_Wv, A_Wo, A_seg_len,
    B_x, B_w_r, B_w_gate, B_w_up, B_w_down, gate_w,
):
    del B_x
    seg = int(A_seg_len)
    batch, n_tok, d_model = A_x.shape
    _, n_heads, d_head = A_Wq.shape
    n_mem = A_mem0.shape[1]
    d_ffn = B_w_gate.shape[1]
    n_seg, n_dt = n_tok // seg, d_model // LANES
    assert (batch, n_seg, seg, d_model, n_mem, d_head) == (1, 64, 32, 1024, 8, LANES)

    hbm = pl.BlockSpec(memory_space=pl.ANY)
    out = pl.pallas_call(
        _kernel,
        out_shape=jax.ShapeDtypeStruct((n_seg, seg, d_model), BF16),
        in_specs=[hbm] * 11,
        out_specs=hbm,
        scratch_shapes=[
            pltpu.VMEM((3, n_heads, d_model // 2, LANES), I32),
            pltpu.VMEM((n_dt, n_heads * LANES, LANES), BF16),
            pltpu.VMEM((3 * n_dt, LANES * n_heads, LANES), BF16),
            pltpu.VMEM((n_dt, n_seg, n_mem, LANES), BF16),
            pltpu.VMEM((3, n_heads, n_seg * n_mem, LANES), F32),
            pltpu.VMEM((n_seg, seg, d_model), BF16),
            pltpu.VMEM((seg // 2, d_model), I32),
            pltpu.VMEM((seg, d_model), F32),
            pltpu.VMEM((n_seg, seg, LANES), F32),
            pltpu.VMEM((n_seg + 1, seg, d_model), BF16),
            pltpu.VMEM((n_mem, d_model), BF16),
            pltpu.VMEM((d_model,), BF16),
            pltpu.VMEM((d_model,), BF16),
            pltpu.VMEM((8, d_model), F32),
            pltpu.VMEM((4, 8, LANES), F32),
            pltpu.VMEM((TOPK, d_model), F32),
            pltpu.VMEM((TOPK, d_ffn), F32),
            pltpu.SMEM((TOPK,), I32),
            pltpu.SemaphoreType.DMA((12,)),
            pltpu.SemaphoreType.REGULAR(()),
        ],
        compiler_params=pltpu.CompilerParams(vmem_limit_bytes=110 * 1024 * 1024),
    )(
        A_x.reshape(n_seg, seg, d_model),
        A_mem0.reshape(n_mem, d_model),
        A_Wq.reshape(n_dt, LANES * n_heads, d_head),
        A_Wk.reshape(n_dt, LANES * n_heads, d_head),
        A_Wv.reshape(n_dt, LANES * n_heads, d_head),
        A_Wo.reshape(n_heads * d_head, d_model),
        B_w_r,
        B_w_gate,
        B_w_up,
        B_w_down,
        gate_w,
    )
    return out.reshape(batch, n_tok, d_model)
```
